```python
import jax
import jax.numpy as jnp

def _softmax(x, axis=-1):
    return jax.nn.softmax(x, axis=axis)
def _gelu(x):
    return jax.nn.gelu(x, approximate=True)
def _silu(x):
    return jax.nn.silu(x)
def _sigmoid(x):
    return jax.nn.sigmoid(x)
def _layernorm(x, axis=-1, eps=1e-5):
    m = jnp.mean(x, axis=axis, keepdims=True)
    v = jnp.var(x, axis=axis, keepdims=True)
    return (x - m) / jnp.sqrt(v + eps)
def _scatter_add(tgt, idx, src, axis=0):
    return tgt.at[idx].add(src)
def _segment_sum(src, seg, n):
    return jax.ops.segment_sum(src, seg, n)
class _Rng:
    def __init__(self, key):
        self._k = key
    def _next(self):
        self._k, sub = jax.random.split(self._k)
        return sub
    def normal(self, shape):
        return jax.random.normal(self._next(), shape, dtype=jnp.bfloat16)
    def randint(self, lo, hi, shape):
        return jax.random.randint(self._next(), shape, lo, hi, dtype=jnp.int32)
    def uniform(self, shape, lo=0.0, hi=1.0):
        return jax.random.uniform(self._next(), shape, jnp.bfloat16, lo, hi)
    def permutation(self, n):
        return jax.random.permutation(self._next(), n)


kernel_name = 'standalone__channel_attn_se__vision'

def _fwd_setup_inputs():
    _rng = _Rng(jax.random.key(int.from_bytes(__import__("os").urandom(4), "little")))
    _w = (lambda a: (lambda t: t.astype(jnp.bfloat16) if jnp.issubdtype(t.dtype, jnp.floating) else t)(jnp.asarray(a)))
    H = W = 384
    C = 96
    r = max(C // 16, 4)
    return {
        "x": _w((lambda *s: _rng.normal(s) * 0.05)(1, H, W, C)),
        "w_down": _w((lambda *s: _rng.normal(s) * 0.05)(C, r)),
        "w_up": _w((lambda *s: _rng.normal(s) * 0.05)(r, C)),
    }

def _fwd_reference(x, w_down, w_up):
    s = x.mean(axis=(1, 2))
    h = _silu(jnp.einsum('bc,cr->br', s, w_down))
    g = _sigmoid(jnp.einsum('br,rc->bc', h, w_up))
    return x * g[:, None, None, :]


def setup_inputs():
    _inp = _fwd_setup_inputs()
    _gk = jax.random.fold_in(jax.random.key(int.from_bytes(__import__("os").urandom(4), "little")), 2**31 - 1)
    _shapes = [[1, 384, 384, 96]]
    _dtypes = ['bfloat16']
    _gks = jax.random.split(_gk, len(_shapes))
    _gs = [jax.random.normal(k, s, dtype=jnp.dtype(d)) * 0.05 for k, s, d in zip(_gks, _shapes, _dtypes)]
    _inp["grad_out"] = _gs[0]
    return _inp

def reference(x, w_down, w_up, grad_out):
    _const = dict()
    def _f(*_d):
        return _fwd_reference(**{'x': _d[0], 'w_down': _d[1], 'w_up': _d[2], **_const})
    _out, _vjp = jax.vjp(_f, x, w_down, w_up)
    _grads = _vjp(grad_out)
    _out0 = jnp.asarray(_out)
    return (_out0, *[jnp.asarray(_g) for _g in _grads])
```

```python
import jax
import jax.numpy as jnp
from jax import lax
import jax.experimental.pallas as pl
import jax.experimental.pallas.tpu as pltpu

F32 = jnp.float32
BF16 = jnp.bfloat16

LANES = 128
SUBLANES = 8
SLAB = 4096
READ_GROUPS = (14, 13)
READ_PIECE = 16
READ_LAG = 64
WRITE_TRIGGER = 8
WRITE_GROUPS = (7, 7, 7, 6)
WRITE_PIECE = 64
LOW, HIGH = 1, 0

SUM_ROWS = 2
READ_DG_ROWS = 1
WRITE_DG_ROWS = 3
WRITE_GX_ROWS = 2


def _spans(sizes):
    starts = [sum(sizes[:i]) for i in range(len(sizes))]
    return list(zip(starts, sizes))


def _make_kernel(H, W, C):
    w_tiles = W // LANES
    c_groups = C // SUBLANES
    rows_per_h = c_groups * w_tiles * SUBLANES
    inv_hw = 1.0 / (H * W)
    read_groups = [(arr, a0, n) for arr in range(2) for a0, n in _spans(READ_GROUPS)]
    write_groups = [(arr, a0, n) for arr in range(2) for a0, n in _spans(WRITE_GROUPS)]
    last = len(read_groups) - 1
    last_high_sem, last_tail_sem = last + 1, last + 2
    reads_per_group = SLAB // READ_PIECE
    writes_per_group = SLAB // WRITE_PIECE
    tail_rows = WRITE_TRIGGER * READ_PIECE

    def kernel(x_hbm, go_hbm, wd_hbm, wu_hbm, out_hbm, gx_hbm, gwd_hbm, gwu_hbm,
               xb, gb, wd_v, wu_v, gwd_v, gwu_v, gate_tab, shift_tab, rsem, wsem, ssem):
        x_rows = xb.reshape(H, rows_per_h, LANES)
        go_rows = gb.reshape(H, rows_per_h, LANES)

        def piece(i, size):
            start = i * size
            return pl.ds(start if isinstance(start, int) else pl.multiple_of(start, size), size)

        def read(arr, slabs, rows, sem):
            src, dst = ((x_hbm, xb), (go_hbm, gb))[arr]
            return pltpu.make_async_copy(src.at[slabs, rows], dst.at[slabs, rows], rsem.at[sem])

        def write(arr, slabs, rows):
            src, dst = ((xb, out_hbm), (gb, gx_hbm))[arr]
            return pltpu.make_async_copy(src.at[slabs, rows], dst.at[slabs, rows], wsem.at[arr])

        def read_issuer(p, i0, low_sem=None):
            arr, a0, n = read_groups[p]
            low_sem = p if low_sem is None else low_sem
            high_sem = last_high_sem if p == last else p

            def issue(i):
                rows = piece(i0 + i, READ_PIECE)
                read(arr, pl.ds(a0, n - 1), rows, low_sem).start(priority=LOW)
                read(arr, pl.ds(a0 + n - 1, 1), rows, high_sem).start(priority=HIGH)
            return issue

        def write_issuer(q, i0):
            arr, a0, n = write_groups[q]
            return lambda i: write(arr, pl.ds(a0, n), piece(i0 + i, WRITE_PIECE)).start()

        def load(ref, h):
            return ref[h].astype(F32).reshape(c_groups, w_tiles, SUBLANES, LANES)

        def table(ref):
            return ref[...].reshape(c_groups, 1, SUBLANES, LANES)

        def sum_row(h, acc):
            return acc + jnp.sum(load(x_rows, h), axis=1)

        def dgate_out_row(h, acc):
            xv = load(x_rows, h)
            acc = acc + jnp.sum(xv * load(go_rows, h), axis=1)
            x_rows[h] = (xv * table(gate_tab)).reshape(rows_per_h, LANES).astype(BF16)
            return acc

        def grad_x_row(h, carry):
            gx = load(go_rows, h) * table(gate_tab) + table(shift_tab)
            go_rows[h] = gx.reshape(rows_per_h, LANES).astype(BF16)
            return carry

        def run(n, issue=None, row_fn=None, h0=0, rows=0, acc=0):
            def body(i, a):
                if issue is not None:
                    issue(i)
                if rows == 1:
                    a = row_fn(h0 + i, a)
                elif rows > 1:
                    a = lax.fori_loop(0, rows, lambda u, b: row_fn(h0 + i * rows + u, b), a)
                return a
            if n == 0:
                return acc
            return body(0, acc) if n == 1 else lax.fori_loop(0, n, body, acc)

        def overlap(n, issuer, i0, row_fn, h0, h1, rows, acc):
            k = min(n, (h1 - h0) // rows)
            acc = run(k, issuer(i0), row_fn, h0, rows, acc)
            run(n - k, issuer(i0 + k))
            return acc, h0 + k * rows

        def lane_sums_as_row(acc):
            a = jnp.concatenate([acc.reshape(C, LANES), jnp.zeros((LANES - C, LANES), F32)], axis=0)
            return jnp.sum(a.T, axis=0, keepdims=True)[:, :C]

        def row_as_table(row):
            r = jnp.concatenate([row, jnp.zeros((1, LANES - C), F32)], axis=1)
            return jnp.broadcast_to(r, (LANES, LANES)).T[:C, :]

        zero = jnp.zeros((c_groups, SUBLANES, LANES), F32)
        wd_copy = pltpu.make_async_copy(wd_hbm, wd_v, ssem.at[0])
        wu_copy = pltpu.make_async_copy(wu_hbm, wu_v, ssem.at[1])

        run(1, read_issuer(0, 0))
        wd_copy.start()
        wu_copy.start()
        run(reads_per_group - 1, read_issuer(0, 1))
        acc, done = zero, 0
        for p in range(1, last + 1):
            arr, a0, n = read_groups[p - 1]
            run(READ_LAG, read_issuer(p, 0))
            read(arr, pl.ds(a0, n), pl.ds(0, SLAB), p - 1).wait()
            ready = (a0 + n) * SLAB // rows_per_h
            steps = reads_per_group - READ_LAG - (WRITE_TRIGGER if p == last else 0)
            row_fn, rows = ((sum_row, SUM_ROWS), (dgate_out_row, READ_DG_ROWS))[arr]
            acc, done = overlap(steps, lambda i0, p=p: read_issuer(p, i0), READ_LAG,
                                row_fn, done, ready, rows, acc)
            if arr == 0 and ready == H:
                assert done == H
                wd_copy.wait()
                wu_copy.wait()
                wd = wd_v[...].astype(F32)
                wu = wu_v[...].astype(F32)
                s = lane_sums_as_row(acc) * inv_hw
                z1 = jnp.sum(wd * s, axis=1, keepdims=True)
                sig1 = jax.nn.sigmoid(z1)
                hidden = z1 * sig1
                z2 = jnp.sum(wu * hidden, axis=0, keepdims=True)
                gate = jax.nn.sigmoid(z2)
                gate_tab[...] = row_as_table(gate)
                acc, done = zero, 0
        run(WRITE_TRIGGER, read_issuer(last, reads_per_group - WRITE_TRIGGER, last_tail_sem))

        def rows_needed(q):
            _, a0, n = write_groups[q]
            return -(-(a0 + n) * SLAB // rows_per_h)

        arr, a0, n = read_groups[last]
        assert done >= rows_needed(0)
        read(arr, pl.ds(a0, n - 1), pl.ds(0, SLAB - tail_rows), last).wait()
        run(writes_per_group, write_issuer(0, 0))
        read(arr, pl.ds(a0 + n - 1, 1), pl.ds(0, SLAB), last_high_sem).wait()
        read(arr, pl.ds(a0, n - 1), pl.ds(SLAB - tail_rows, tail_rows), last_tail_sem).wait()

        lead = rows_needed(1) + (H - rows_needed(1)) % WRITE_DG_ROWS
        acc = run(lead - done, None, dgate_out_row, done, 1, acc)
        acc, done = overlap(writes_per_group, lambda i0: write_issuer(1, i0), 0,
                            dgate_out_row, lead, H, WRITE_DG_ROWS, acc)
        assert done == H

        dgate = lane_sums_as_row(acc)
        dz2 = dgate * (gate * (1.0 - gate))
        gwu_v[...] = (hidden * dz2).astype(BF16)
        dhidden = jnp.sum(wu * dz2, axis=1, keepdims=True)
        dz1 = dhidden * sig1 + (z1 * dhidden) * (sig1 * (1.0 - sig1))
        gwd_v[...] = (dz1 * s).astype(BF16)
        ds = jnp.sum(wd * dz1, axis=0, keepdims=True)
        shift_tab[...] = row_as_table(ds * inv_hw)
        gwd_copy = pltpu.make_async_copy(gwd_v, gwd_hbm, ssem.at[2])
        gwu_copy = pltpu.make_async_copy(gwu_v, gwu_hbm, ssem.at[3])
        gwd_copy.start()
        gwu_copy.start()

        done = 0
        for q in range(2, len(write_groups)):
            assert write_groups[q][0] == 0 or done >= rows_needed(q)
            _, done = overlap(writes_per_group, lambda i0, q=q: write_issuer(q, i0), 0,
                              grad_x_row, done, H, WRITE_GX_ROWS, 0)

        gwd_copy.wait()
        gwu_copy.wait()
        pltpu.make_async_copy(xb, out_hbm, wsem.at[0]).wait()
        pltpu.make_async_copy(gb, gx_hbm, wsem.at[1]).wait()

    return kernel, len(read_groups) + 2


@jax.jit
def pallas_standalone__channel_attn_se__vision_kernel(
    x: jax.Array,
    w_down: jax.Array,
    w_up: jax.Array,
    grad_out: jax.Array,
):
    B, H, W, C = x.shape
    R = w_up.shape[0]
    w_tiles, c_groups = W // LANES, C // SUBLANES
    n_slabs = H * W * C // (LANES * SLAB)
    assert B == 1 and w_tiles * LANES == W and c_groups * SUBLANES == C and C <= LANES
    assert n_slabs * SLAB * LANES == H * W * C
    assert n_slabs == sum(READ_GROUPS) == sum(WRITE_GROUPS)

    def to_slabs(a):
        a = a.reshape(H, w_tiles, LANES, c_groups, SUBLANES).transpose(0, 3, 1, 4, 2)
        return a.reshape(n_slabs, SLAB, LANES)

    def from_slabs(a):
        a = a.reshape(H, c_groups, w_tiles, SUBLANES, LANES).transpose(0, 2, 4, 1, 3)
        return a.reshape(B, H, W, C)

    kernel, n_read_sems = _make_kernel(H, W, C)
    big = jax.ShapeDtypeStruct((n_slabs, SLAB, LANES), BF16)
    small = jax.ShapeDtypeStruct((R, C), BF16)
    hbm = pl.BlockSpec(memory_space=pl.ANY)
    out, grad_x, grad_w_down_t, grad_w_up = pl.pallas_call(
        kernel,
        in_specs=[hbm] * 4,
        out_specs=[hbm] * 4,
        out_shape=[big, big, small, small],
        scratch_shapes=[
            pltpu.VMEM(big.shape, BF16),
            pltpu.VMEM(big.shape, BF16),
            pltpu.VMEM(small.shape, BF16),
            pltpu.VMEM(small.shape, BF16),
            pltpu.VMEM(small.shape, BF16),
            pltpu.VMEM(small.shape, BF16),
            pltpu.VMEM((C, LANES), F32),
            pltpu.VMEM((C, LANES), F32),
            pltpu.SemaphoreType.DMA((n_read_sems,)),
            pltpu.SemaphoreType.DMA((2,)),
            pltpu.SemaphoreType.DMA((4,)),
        ],
        compiler_params=pltpu.CompilerParams(
            vmem_limit_bytes=64 * 1024 * 1024,
            disable_bounds_checks=True,
            disable_semaphore_checks=True,
        ),
    )(to_slabs(x), to_slabs(grad_out), w_down.T, w_up)
    return from_slabs(out), from_slabs(grad_x), grad_w_down_t.T, grad_w_up
```

```python
import jax
import jax.numpy as jnp
from jax import lax
import jax.experimental.pallas as pl
import jax.experimental.pallas.tpu as pltpu

F32 = jnp.float32
BF16 = jnp.bfloat16

LANES = 128
SUBLANES = 8
SLAB = 4096
PIECE = 16
LOW, HIGH = 1, 0

READ_GROUPS = (13, 14)
READ_LAG = 64
TAIL_STEPS = 2
TAIL_PIECE = 8

WRITE_GROUPS = (7, 7, 7, 6)
WRITES_PER_STEP = 4
WRITE_LEAD = 16

SUM_ROWS = 2
READ_DG_ROWS = 1
WRITE_DG_ROWS = 2
WRITE_GX_ROWS = 2


def _spans(sizes):
    starts = [sum(sizes[:i]) for i in range(len(sizes))]
    return list(zip(starts, sizes))


def _make_kernel(H, W, C):
    w_tiles = W // LANES
    c_groups = C // SUBLANES
    rows_per_h = c_groups * w_tiles * SUBLANES
    inv_hw = 1.0 / (H * W)
    read_groups = [(arr, a0, n) for arr in range(2) for a0, n in _spans(READ_GROUPS)]
    write_groups = [(arr, a0, n) for arr in range(2) for a0, n in _spans(WRITE_GROUPS)]
    last = len(read_groups) - 1
    read_steps = SLAB // PIECE
    write_steps = SLAB // (PIECE * WRITES_PER_STEP)
    tail_rows = TAIL_STEPS * PIECE

    def kernel(x_hbm, go_hbm, wd_hbm, wu_hbm, out_hbm, gx_hbm, gwd_hbm, gwu_hbm,
               xb, gb, wd_v, wu_v, gwd_v, gwu_v, gate_tab, shift_tab, rsem, wsem, ssem):
        x_rows = xb.reshape(H, rows_per_h, LANES)
        go_rows = gb.reshape(H, rows_per_h, LANES)

        def piece(i, size):
            start = i * size
            return pl.ds(start if isinstance(start, int) else pl.multiple_of(start, size), size)

        def read(p, slab0, n_slabs, rows):
            arr, a0, _ = read_groups[p]
            src, dst = ((x_hbm, xb), (go_hbm, gb))[arr]
            slabs = pl.ds(a0 + slab0, n_slabs)
            return pltpu.make_async_copy(src.at[slabs, rows], dst.at[slabs, rows], rsem.at[p])

        def read_issuer(p, i0):
            n = read_groups[p][2]

            def issue(i):
                rows = piece(i0 + i, PIECE)
                read(p, 0, n - 1, rows).start(priority=LOW)
                read(p, n - 1, 1, rows).start(priority=HIGH)
            return issue

        def wait_reads(p):
            _, a0, n = read_groups[p]
            read(p, 0, n, pl.ds(0, SLAB)).wait()
            return (a0 + n) * SLAB // rows_per_h

        def write_issuer(q, i0):
            arr, a0, n = write_groups[q]
            src, dst = ((xb, out_hbm), (gb, gx_hbm))[arr]

            def issue(i):
                for j in range(WRITES_PER_STEP):
                    idx = (pl.ds(a0, n), piece((i0 + i) * WRITES_PER_STEP + j, PIECE))
                    pltpu.make_async_copy(src.at[idx], dst.at[idx], wsem.at[arr]).start()
            return issue

        def rows_written_by(q):
            _, a0, n = write_groups[q]
            return -(-(a0 + n) * SLAB // rows_per_h)

        def load(ref, h):
            return ref[h].astype(F32).reshape(c_groups, w_tiles, SUBLANES, LANES)

        def table(ref):
            return ref[...].reshape(c_groups, 1, SUBLANES, LANES)

        def sum_row(h, acc):
            return acc + jnp.sum(load(x_rows, h), axis=1)

        def dgate_out_row(h, acc):
            xv = load(x_rows, h)
            acc = acc + jnp.sum(xv * load(go_rows, h), axis=1)
            x_rows[h] = (xv * table(gate_tab)).reshape(rows_per_h, LANES).astype(BF16)
            return acc

        def grad_x_row(h, carry):
            gx = load(go_rows, h) * table(gate_tab) + table(shift_tab)
            go_rows[h] = gx.reshape(rows_per_h, LANES).astype(BF16)
            return carry

        def run(n, issue, row_fn=None, h0=0, rows=0, acc=0):
            def body(i, a):
                issue(i)
                if rows == 1:
                    a = row_fn(h0 + i, a)
                elif rows > 1:
                    a = lax.fori_loop(0, rows, lambda u, b: row_fn(h0 + i * rows + u, b), a)
                return a
            if n == 0:
                return acc
            return body(0, acc) if n == 1 else lax.fori_loop(0, n, body, acc)

        def overlap(issuer, group, i0, i1, row_fn, h0, h1, rows, acc):
            k = min(i1 - i0, (h1 - h0) // rows)
            acc = run(k, issuer(group, i0), row_fn, h0, rows, acc)
            run(i1 - i0 - k, issuer(group, i0 + k))
            return acc, h0 + k * rows

        def lane_sums_as_row(acc):
            a = jnp.concatenate([acc.reshape(C, LANES), jnp.zeros((LANES - C, LANES), F32)], axis=0)
            return jnp.sum(a.T, axis=0, keepdims=True)[:, :C]

        def row_as_table(row):
            r = jnp.concatenate([row, jnp.zeros((1, LANES - C), F32)], axis=1)
            return jnp.broadcast_to(r, (LANES, LANES)).T[:C, :]

        zero = jnp.zeros((c_groups, SUBLANES, LANES), F32)
        wd_copy = pltpu.make_async_copy(wd_hbm, wd_v, ssem.at[0])
        wu_copy = pltpu.make_async_copy(wu_hbm, wu_v, ssem.at[1])

        run(1, read_issuer(0, 0))
        wd_copy.start()
        wu_copy.start()
        run(read_steps - 1, read_issuer(0, 1))
        acc, done = zero, 0
        for p in range(1, last + 1):
            run(READ_LAG, read_issuer(p, 0))
            ready = wait_reads(p - 1)
            summing_x = read_groups[p - 1][0] == 0
            row_fn, rows = (sum_row, SUM_ROWS) if summing_x else (dgate_out_row, READ_DG_ROWS)
            end = read_steps - (TAIL_STEPS if p == last else 0)
            acc, done = overlap(read_issuer, p, READ_LAG, end, row_fn, done, ready, rows, acc)
            if summing_x and ready == H:
                assert done == H
                wd_copy.wait()
                wu_copy.wait()
                wd = wd_v[...].astype(F32)
                wu = wu_v[...].astype(F32)
                s = lane_sums_as_row(acc) * inv_hw
                z1 = jnp.sum(wd * s, axis=1, keepdims=True)
                sig1 = jax.nn.sigmoid(z1)
                hidden = z1 * sig1
                z2 = jnp.sum(wu * hidden, axis=0, keepdims=True)
                gate = jax.nn.sigmoid(z2)
                gate_tab[...] = row_as_table(gate)
                acc, done = zero, 0

        n_low = read_groups[last][2] - 1
        read(last, n_low, 1, pl.ds(SLAB - tail_rows, tail_rows)).start(priority=HIGH)

        def issue_tail(i):
            rows = piece((SLAB - tail_rows) // TAIL_PIECE + i, TAIL_PIECE)
            for slab in range(n_low):
                read(last, slab, 1, rows).start(priority=LOW)
        run(tail_rows // TAIL_PIECE, issue_tail)

        assert done >= rows_written_by(0)
        run(WRITE_LEAD, write_issuer(0, 0))
        wait_reads(last)
        acc, done = overlap(write_issuer, 0, WRITE_LEAD, write_steps,
                            dgate_out_row, done, H, WRITE_DG_ROWS, acc)
        assert done >= rows_written_by(1)
        acc, done = overlap(write_issuer, 1, 0, write_steps,
                            dgate_out_row, done, H, WRITE_DG_ROWS, acc)
        assert done == H

        dgate = lane_sums_as_row(acc)
        dz2 = dgate * (gate * (1.0 - gate))
        gwu_v[...] = (hidden * dz2).astype(BF16)
        dhidden = jnp.sum(wu * dz2, axis=1, keepdims=True)
        dz1 = dhidden * sig1 + (z1 * dhidden) * (sig1 * (1.0 - sig1))
        gwd_v[...] = (dz1 * s).astype(BF16)
        ds = jnp.sum(wd * dz1, axis=0, keepdims=True)
        shift_tab[...] = row_as_table(ds * inv_hw)
        gwd_copy = pltpu.make_async_copy(gwd_v, gwd_hbm, ssem.at[2])
        gwu_copy = pltpu.make_async_copy(gwu_v, gwu_hbm, ssem.at[3])
        gwd_copy.start()
        gwu_copy.start()

        done = 0
        for q in range(2, len(write_groups)):
            assert write_groups[q][0] == 0 or done >= rows_written_by(q)
            _, done = overlap(write_issuer, q, 0, write_steps,
                              grad_x_row, done, H, WRITE_GX_ROWS, 0)

        gwd_copy.wait()
        gwu_copy.wait()
        pltpu.make_async_copy(xb, out_hbm, wsem.at[0]).wait()
        pltpu.make_async_copy(gb, gx_hbm, wsem.at[1]).wait()

    return kernel


@jax.jit
def pallas_standalone__channel_attn_se__vision_kernel(
    x: jax.Array,
    w_down: jax.Array,
    w_up: jax.Array,
    grad_out: jax.Array,
):
    B, H, W, C = x.shape
    R = w_up.shape[0]
    w_tiles, c_groups = W // LANES, C // SUBLANES
    n_slabs = H * W * C // (LANES * SLAB)
    assert B == 1 and w_tiles * LANES == W and c_groups * SUBLANES == C and C <= LANES
    assert n_slabs * SLAB * LANES == H * W * C
    assert n_slabs == sum(READ_GROUPS) == sum(WRITE_GROUPS)

    def to_slabs(a):
        a = a.reshape(H, w_tiles, LANES, c_groups, SUBLANES).transpose(0, 3, 1, 4, 2)
        return a.reshape(n_slabs, SLAB, LANES)

    def from_slabs(a):
        a = a.reshape(H, c_groups, w_tiles, SUBLANES, LANES).transpose(0, 2, 4, 1, 3)
        return a.reshape(B, H, W, C)

    big = jax.ShapeDtypeStruct((n_slabs, SLAB, LANES), BF16)
    small = jax.ShapeDtypeStruct((R, C), BF16)
    hbm = pl.BlockSpec(memory_space=pl.ANY)
    out, grad_x, grad_w_down_t, grad_w_up = pl.pallas_call(
        _make_kernel(H, W, C),
        in_specs=[hbm] * 4,
        out_specs=[hbm] * 4,
        out_shape=[big, big, small, small],
        scratch_shapes=[
            pltpu.VMEM(big.shape, BF16),
            pltpu.VMEM(big.shape, BF16),
            pltpu.VMEM(small.shape, BF16),
            pltpu.VMEM(small.shape, BF16),
            pltpu.VMEM(small.shape, BF16),
            pltpu.VMEM(small.shape, BF16),
            pltpu.VMEM((C, LANES), F32),
            pltpu.VMEM((C, LANES), F32),
            pltpu.SemaphoreType.DMA((2 * len(READ_GROUPS),)),
            pltpu.SemaphoreType.DMA((2,)),
            pltpu.SemaphoreType.DMA((4,)),
        ],
        compiler_params=pltpu.CompilerParams(
            vmem_limit_bytes=64 * 1024 * 1024,
            disable_bounds_checks=True,
            disable_semaphore_checks=True,
        ),
    )(to_slabs(x), to_slabs(grad_out), w_down.T, w_up)
    return from_slabs(out), from_slabs(grad_x), grad_w_down_t.T, grad_w_up
```
